```python
import os as _os
_os.environ.setdefault("JAX_PLATFORMS", "cpu")
import jax
import jax.numpy as jnp

def _softmax(x, axis=-1):
    return jax.nn.softmax(x, axis=axis)
def _gelu(x):
    return jax.nn.gelu(x, approximate=True)
def _silu(x):
    return jax.nn.silu(x)
def _sigmoid(x):
    return jax.nn.sigmoid(x)
def _layernorm(x, axis=-1, eps=1e-5):
    m = jnp.mean(x, axis=axis, keepdims=True)
    v = jnp.var(x, axis=axis, keepdims=True)
    return (x - m) / jnp.sqrt(v + eps)
def _scatter_add(tgt, idx, src, axis=0):
    return tgt.at[idx].add(src)
def _segment_sum(src, seg, n):
    return jax.ops.segment_sum(src, seg, n)
class _Rng:
    def __init__(self, key):
        self._k = key
    def _next(self):
        self._k, sub = jax.random.split(self._k)
        return sub
    def normal(self, shape):
        return jax.random.normal(self._next(), shape, dtype=jnp.bfloat16)
    def randint(self, lo, hi, shape):
        return jax.random.randint(self._next(), shape, lo, hi, dtype=jnp.int32)
    def uniform(self, shape, lo=0.0, hi=1.0):
        return jax.random.uniform(self._next(), shape, jnp.bfloat16, lo, hi)
    def permutation(self, n):
        return jax.random.permutation(self._next(), n)


kernel_name = 'sequential_preLN__softmax_full_mha__dense_activation_squared_relu__prompt'

def setup_inputs():
    _rng = _Rng(jax.random.key(int.from_bytes(__import__("os").urandom(4), "little")))
    _w = (lambda a: (lambda t: t.astype(jnp.bfloat16) if jnp.issubdtype(t.dtype, jnp.floating) else t)(jnp.asarray(a)))
    def _A_setup():
        B, S, D = 1, 2048, 448
        return {
            "x": _w((lambda *s: _rng.normal(s) * 0.05)(B, S, D)),
            "wqkv": _w((lambda *s: _rng.normal(s) * 0.05)(D, 3 * D)),
            "wo": _w((lambda *s: _rng.normal(s) * 0.05)(D, D)),
        }
    _A_in = _A_setup()

    def _B_setup():
        B, S, D, F = 1, 2048, 448, 1792
        return {
            "x": _w((lambda *s: _rng.normal(s) * 0.05)(B, S, D)),
            "w1": _w((lambda *s: _rng.normal(s) * 0.05)(D, F)),
            "b1": _w((lambda *s: _rng.normal(s) * 0.05)(F)),
            "w2": _w((lambda *s: _rng.normal(s) * 0.05)(F, D)),
            "b2": _w((lambda *s: _rng.normal(s) * 0.05)(D)),
        }
    _B_in = _B_setup()

    return {
        "A_x": _A_in["x"],
        "A_wqkv": _A_in["wqkv"],
        "A_wo": _A_in["wo"],
        "B_x": _B_in["x"],
        "B_w1": _B_in["w1"],
        "B_b1": _B_in["b1"],
        "B_w2": _B_in["w2"],
        "B_b2": _B_in["b2"],
    }

def reference(A_x, A_wqkv, A_wo, B_x, B_w1, B_b1, B_w2, B_b2):
    def _A_ref(x, wqkv, wo):
        B, S, D = x.shape
        H = 16; Dh = D // H
        qkv = (lambda x, *d: x.transpose(*d))((x @ wqkv).reshape(B, S, 3, H, Dh), 2, 0, 3, 1, 4)
        q, k, v = qkv[0], qkv[1], qkv[2]
        scale = Dh ** -0.5
        scores = jnp.einsum("bhqd,bhkd->bhqk", q, k) * scale
        p = _softmax(scores, axis=-1)
        o = jnp.einsum("bhqk,bhkd->bhqd", p, v)
        return (lambda x, *d: x.transpose(*d))(o, 0, 2, 1, 3).reshape(B, S, D) @ wo

    def _B_ref(x, w1, b1, w2, b2):
        h = jnp.einsum("bsd,df->bsf", x, w1) + b1
        zero = jnp.zeros_like(h)
        r = jnp.where(h > zero, h, zero)
        h = r * r
        out = jnp.einsum("bsf,fd->bsd", h, w2) + b2
        return out

    x = A_x
    h = x + _A_ref(_layernorm(x, axis=-1), A_wqkv, A_wo)
    h2 = h + _B_ref(_layernorm(h, axis=-1), B_w1, B_b1, B_w2, B_b2)
    return h2
```

```python
import math
import jax
import jax.numpy as jnp
from jax import lax
import jax.experimental.pallas as pl
import jax.experimental.pallas.tpu as pltpu

H = 16
EPS = 1e-5
BN1 = 512
BQ = 512
CK = 256
BN3 = 512
F32, BF16, U32 = jnp.float32, jnp.bfloat16, jnp.uint32


def _ln_t(x):
    m = jnp.mean(x, axis=0, keepdims=True)
    c = x - m
    v = jnp.mean(c * c, axis=0, keepdims=True)
    return c * lax.rsqrt(v + EPS)


def _pk(x):
    return pltpu.bitcast(x, jnp.uint32)


def _up(x):
    return pltpu.bitcast(x, BF16)


def _dot(a, b):
    return jnp.dot(a, b, preferred_element_type=F32)


def _kernel(xT_ref, wqkv_ref, wo_ref, w1_ref, b1_ref, w2T_ref, b2_ref, outT_ref,
            wqkvT, woT, w1T, b2c, qT, kn, vT, sA, sB, oT):
    D, S = xT_ref.shape
    F = w1_ref.shape[1]
    Dh = D // H
    G = 4 * Dh
    qscale = Dh ** -0.5 * math.log2(math.e)

    pad = 512 - D
    for j in range(0, 3 * D, 128):
        w = min(128, 3 * D - j)
        blk = wqkv_ref[:, j:j + w]
        wqkvT[j // 2:(j + w) // 2, :] = _pk(blk.astype(F32).T.astype(BF16))
    woT[...] = _pk(wo_ref[...].astype(F32).T.astype(BF16))
    b1 = b1_ref[...].astype(F32)
    row = lax.broadcasted_iota(jnp.int32, (pad, F), 0)
    w1a = jnp.concatenate([w1_ref[...].astype(F32), jnp.where(row == 0, b1, 0.0)], axis=0)
    w1T[...] = _pk(w1a.T.astype(BF16))
    b2c[...] = jnp.broadcast_to(b2_ref[...].astype(F32), (128, D)).T

    def p1(i, c):
        n0 = pl.multiple_of(i * BN1, BN1)
        xn = _ln_t(xT_ref[:, pl.ds(n0, BN1)].astype(F32)).astype(BF16)
        q = _dot(_up(wqkvT[0:D // 2, :]), xn) * qscale
        qT[:, pl.ds(n0, BN1)] = _pk(q.astype(BF16))
        k = _dot(_up(wqkvT[D // 2:D, :]), xn)
        for g in range(4):
            kg = jnp.concatenate([k[G * g:G * (g + 1)], jnp.zeros((128 - G, BN1), F32)], axis=0)
            kn[g, pl.ds(pl.multiple_of(i * (BN1 // 2), BN1 // 2), BN1 // 2), :] = _pk(kg.T.astype(BF16))
        v = _dot(_up(wqkvT[D:3 * D // 2, :]), xn)
        r = lax.broadcasted_iota(jnp.int32, (32, BN1), 0)
        for h in range(H):
            if h % 2 == 0:
                vh = jnp.where(r < Dh, v[Dh * h:Dh * h + 32], 1.0)
            else:
                vh = jnp.where(r >= 32 - Dh, v[Dh * (h + 1) - 32:Dh * (h + 1)], 1.0)
            vT[h, :, pl.ds(n0, BN1)] = _pk(vh.astype(BF16))
        return c
    lax.fori_loop(0, S // BN1, p1, 0)

    NQ = S // BQ
    def q_tile(g, j, q0):
        lo, hi = Dh // 2 * j, Dh // 2 * (j + 1)
        a, b = lo // 8 * 8, -(-hi // 8) * 8
        qg = qT[pl.ds(pl.multiple_of(g * (G // 2) + a, 8), b - a), pl.ds(q0, BQ)]
        r = lax.broadcasted_iota(jnp.int32, (b - a, BQ), 0) + a
        qg = jnp.where((r >= lo) & (r < hi), qg, jnp.uint32(0))
        parts = ([jnp.zeros((a, BQ), jnp.uint32)] if a else []) + [qg, jnp.zeros((64 - b, BQ), jnp.uint32)]
        return _up(jnp.concatenate(parts, axis=0))

    def step(s_w, gq, jq, q0, s_r, m_r, hv, off=0):
        m = acc = None
        if s_w is not None:
            qm = q_tile(gq, jq, q0)
        for c in range(0, S, CK):
            if s_w is not None:
                s = _dot(_up(kn[gq, c // 2:(c + CK) // 2, :]), qm)
                s_w[c:c + CK, :] = s
                mc = jnp.max(s.reshape(CK // 8, 8, BQ), axis=0)
                m = mc if m is None else jnp.maximum(m, mc)
            if s_r is not None:
                p = jnp.exp2(s_r[pl.ds(off + c, CK), :] - m_r).astype(BF16)
                pv = _dot(_up(vT[hv, :, c:c + CK]), p)
                acc = pv if acc is None else acc + pv
        if m is not None:
            m = jnp.max(m, axis=0, keepdims=True)
        return m, acc

    def p2(t, m):
        qb, g = t // 4, t % 4
        q0 = pl.multiple_of(qb * BQ, BQ)
        tn = jnp.minimum(t + 1, 4 * NQ - 1)
        outs = []
        off = pl.multiple_of((t // 1024) * 8, 8)
        for j in range(4):
            s_r, s_w = (sA, sB) if j % 2 == 0 else (sB, sA)
            if j < 3:
                m, acc = step(s_w, g, j + 1, q0, s_r, m, 4 * g + j, off)
            else:
                m, acc = step(s_w, tn % 4, 0, pl.multiple_of((tn // 4) * BQ, BQ), s_r, m, 4 * g + j, off)
            l = acc[31:32] if j % 2 == 0 else acc[0:1]
            outs.append(acc * (1.0 / l))
        r = lax.broadcasted_iota(jnp.int32, (8, BQ), 0)
        parts = []
        for j in (0, 2):
            parts += [outs[j][0:24], jnp.where(r < 4, outs[j][24:32], outs[j + 1][0:8]), outs[j + 1][8:32]]
        oT[pl.ds(pl.multiple_of(g * (G // 2), 8), G // 2), pl.ds(q0, BQ)] = _pk(jnp.concatenate(parts, axis=0).astype(BF16))
        return m
    m0, _ = step(sA, 0, 0, 0, None, None, None)
    lax.fori_loop(0, 4 * NQ, p2, m0)

    def p3(i, c):
        n0 = pl.multiple_of(i * BN3, BN3)
        h = xT_ref[:, pl.ds(n0, BN3)].astype(F32) + _dot(_up(woT[...]), _up(oT[:, pl.ds(n0, BN3)]))
        r = lax.broadcasted_iota(jnp.int32, (pad, BN3), 0)
        hn = jnp.concatenate([_ln_t(h), jnp.where(r == 0, 1.0, 0.0)], axis=0).astype(BF16)
        u = jnp.maximum(_dot(_up(w1T[...]), hn), 0.0)
        y = _dot(w2T_ref[...], (u * u).astype(BF16))
        outT_ref[:, pl.ds(n0, BN3)] = (y + h + jnp.tile(b2c[...], (1, BN3 // 128))).astype(outT_ref.dtype)
        return c
    lax.fori_loop(0, S // BN3, p3, 0)


@jax.jit
def pallas_sequential_preLN__softmax_full_mha__dense_activation_squared_relu__prompt_kernel(
    A_x, A_wqkv, A_wo, B_x, B_w1, B_b1, B_w2, B_b2,
):
    del B_x
    B, S, D = A_x.shape
    F = B_w1.shape[1]
    outT = pl.pallas_call(
        _kernel,
        out_shape=jax.ShapeDtypeStruct((D, S), A_x.dtype),
        scratch_shapes=[
            pltpu.VMEM((3 * D // 2, D), U32), pltpu.VMEM((D // 2, D), U32), pltpu.VMEM((F // 2, 512), U32),
            pltpu.VMEM((D, 128), F32),
            pltpu.VMEM((D // 2, S), U32), pltpu.VMEM((4, S // 2, 128), U32), pltpu.VMEM((H, 16, S), U32),
            pltpu.VMEM((S, BQ), F32), pltpu.VMEM((S, BQ), F32), pltpu.VMEM((D // 2, S), U32),
        ],
        compiler_params=pltpu.CompilerParams(vmem_limit_bytes=100 * 1024 * 1024),
        name="block",
    )(A_x.reshape(S, D).T, A_wqkv, A_wo, B_w1, B_b1.reshape(1, F), B_w2.T, B_b2.reshape(1, D))
    return outT.T.reshape(B, S, D)
```

```python
import itertools
import math

import jax
import jax.numpy as jnp
from jax import lax
import jax.experimental.pallas as pl
import jax.experimental.pallas.tpu as pltpu

H = 16
EPS = 1e-5
BN = 512
CK = 128
U = 15
TK = 3
L_LO, L_HI = 2.0 ** -40, 2.0 ** 60
F32, BF16, U32, I32 = jnp.float32, jnp.bfloat16, jnp.uint32, jnp.int32

PH = '23'
OS = 1
XS = 1
XT = 2
PA = 3
PB = 1
SL = -1
BR = 2
TR = 1
MN = 1
FULL_AT = 14
ORD0 = (4, 7, 3, 5, 1, 2, 6)
ORD1 = (2, 4, 5, 3, 7, 1, 6)
ORD2 = (5, 3, 2, 4, 1, 6, 7)
XH = 5
TW = 128
RB = 0
WR = 1
HO3 = (3, 4, 1, 2, 11, 9, 10, 5, 15, 14, 12, 13, 8, 7, 6, 17, 16, 21, 18, 19, 20, 24, 25, 22, 26, 23)
HO4 = (26, 1, 11, 2, 4, 3, 9, 14, 8, 22, 19, 17, 10, 5, 7, 20, 23, 18, 25, 6, 12, 16, 13, 24, 21, 15)

_STRASSEN = {
    1: ((11, 22), (11, 22), (11, 22)),
    2: ((21, 22), (11,), (21, -22)),
    3: ((11,), (12, -22), (12, 22)),
    4: ((22,), (21, -11), (11, 21)),
    5: ((11, 12), (22,), (-11, 12)),
    6: ((21, -11), (11, 12), (22,)),
    7: ((12, -22), (21, 22), (11,)),
}
_HK = {
    1: ((11,), (11,)), 2: ((12,), (21,)), 3: ((21,), (12, -22)), 4: ((21, 22), (22,)),
    5: ((31,), (13, -23)), 6: ((31, 32), (23,)), 7: ((42,), (24, -14)), 8: ((41, 42), (14,)),
    9: ((21, 22, 12), (11, 12, -22)), 10: ((12, 22), (11, 12, -22, -21)), 11: ((21, 22, 12, 11), (11, 12)),
    12: ((31, 32, 12), (11, 13, -23)), 13: ((12, 32), (11, 13, -23, -21)), 14: ((31, 32, 12, 11), (11, 13)),
    15: ((41, 42, 11), (21, -24, 14)), 16: ((11, 41), (21, -24, 14, -11)), 17: ((41, 42, 11, 12), (21, -24)),
    18: ((21, 42), (14, 22)), 19: ((41, -21), (12, 14)), 20: ((22, -42), (22, 24)),
    21: ((31, 42), (14, 23)), 22: ((41, -31), (13, 14)), 23: ((32, -42), (23, 24)),
    24: ((12, 22, -31), (11, 12, 23)), 25: ((12, 22, 32), (21, 22, 23)), 26: ((11, 21, 31), (11, 12, 13)),
}
_HK_OUT = {
    11: (1, 2), 22: (3, 4), 33: (5, 6), 44: (7, 8),
    21: (9, -2, -3, -10), 12: (11, -9, -1, -4), 31: (12, -2, -5, -13), 13: (14, -12, -1, -6),
    41: (15, 7, -1, -16), 14: (15, 2, -8, -17), 42: (18, 3, -8, 19), 24: (18, 7, -4, 20),
    43: (21, 5, -8, 22), 34: (21, 7, -6, 23), 32: (10, -24, -6, -131, 25), 23: (24, -11, -5, -113, 26),
}


def _pk(x):
    return pltpu.bitcast(x, U32)


def _up(x):
    return pltpu.bitcast(x, BF16)


def _dot(a, b):
    return lax.dot_general(a, b, (((1,), (0,)), ((), ())), preferred_element_type=F32)


def _rows(parts):
    return jnp.concatenate(parts, axis=0)


def _blocks(c):
    return _rows([jnp.concatenate(r, axis=1) for r in c])


def _signed_sum(get, terms):
    out = get(terms[0])
    for t in terms[1:]:
        out = out + get(t) if t > 0 else out - get(-t)
    return out


def _ln_stats(load, d, n, true, slow=False):
    mean, rstd = [], []
    for j in range(0, n, 128):
        acc = load(0, j)
        if rstd and true is not None:
            acc = jnp.where(true, acc, rstd[-1])
        for r in range(8, d, 8):
            acc = acc + load(r, j)
        m = jnp.broadcast_to(jnp.sum(acc, axis=0, keepdims=True) * (1.0 / d), (8, 128))
        acc = None
        for r in range(0, d, 8):
            x = load(r, j)
            if slow and r:
                x = jnp.where(true, x, acc)
            c = x - m
            acc = c * c if acc is None else acc + c * c
        v = jnp.broadcast_to(jnp.sum(acc, axis=0, keepdims=True) * (1.0 / d), (8, 128))
        mean.append(m)
        rstd.append(lax.rsqrt(v + EPS))
    return jnp.concatenate(mean, axis=1), jnp.concatenate(rstd, axis=1)


def _ln_apply(load, d, stats):
    return _rows([(load(r) - stats[0]) * stats[1] for r in range(0, d, 8)])


def _strassen(a_ref, b, order, hooks=None):
    k, n = b.shape[0] // 2, b.shape[1] // 2
    bq = {11: b[:k, :n], 12: b[:k, n:], 21: b[k:, :n], 22: b[k:, n:]}
    c = {}
    for i in order:
        lhs, rhs, dst = _STRASSEN[i]
        rhs = _signed_sum(bq.get, rhs)
        if hooks and i in hooks:
            hooks[i]()
        m = _dot(_signed_sum(lambda q: a_ref[q // 10 - 1, q % 10 - 1], lhs), rhs)
        for t in dst:
            if abs(t) not in c:
                c[abs(t)] = (m, t > 0)
            else:
                acc, pos = c[abs(t)]
                c[abs(t)] = (m + acc if pos and t > 0 else acc - m if pos else m - acc, True)
    return [[c[11][0], c[12][0]], [c[21][0], c[22][0]]]


def _hopcroft_kerr(a, b, order, act=lambda x, r: x, true=None):
    k, n = b.shape[0] // 2, b.shape[1] // 4
    memo = {}

    def rhs(terms, r, prev):
        def tie(x):
            nonlocal prev
            if prev is not None and true is not None:
                x, prev = jnp.where(true, x, prev), None
            return x

        for t in terms:
            q = abs(t)
            if ((q,), r) not in memo:
                r0 = (q // 10 - 1) * k + r
                memo[(q,), r] = act(tie(b[r0:r0 + 8, (q % 10 - 1) * n:q % 10 * n]), r0)
        for c in range(2, len(terms) + 1):
            if (terms[:c], r) not in memo:
                f, t = tie(memo[terms[:c - 1], r]), terms[c - 1]
                memo[terms[:c], r] = f + memo[(t,), r] if t > 0 else f - memo[(-t,), r]
        return memo[terms, r]

    m = {}
    for i in order:
        rows = []
        for r in reversed(range(0, k, 8)):
            rows.append(rhs(_HK[i][1], r, rows[-1] if rows and r % TW != TW - 8 else None))
        m[i] = _dot(a(i), _rows(rows[::-1]).astype(BF16 if RB and true is not None else F32))
        for q, terms in _HK_OUT.items():
            if 100 + q not in m and all(abs(t) in m for t in terms):
                rest = sorted((t for t in terms if t != i), key=lambda t: t < 0)
                if i in terms and rest[0] > 0:
                    m[100 + q] = m[i] + _signed_sum(m.get, rest)
                else:
                    m[100 + q] = _signed_sum(m.get, terms)
    return _blocks([[m[100 + 10 * r + c] for c in range(1, 5)] for r in range(1, 5)])


def _kernel(*refs):
    lax.while_loop(lambda attempt: attempt < 2, lambda attempt: _block(attempt, *refs), 0)


def _block(attempt, x_hbm, wqkv_hbm, wo_hbm, w1_hbm, b1_hbm, w2T_hbm, b2_hbm, out_hbm,
            kb0, kb1, sv, qp, qf, kn, vT, of, sl, ku, xT, outT, wo, aqkv, ao, a1, t1, b1c, hs,
            w1, w2T, a2, b2c, wqkv, b1, b2, sem_x, sem_w, sem_o):
    D, S = x_hbm.shape
    F = w1_hbm.shape[1]
    Dh, D2, D4, F2, F4 = D // H, D // 2, D // 4, F // 2, F // 4
    NB, NC, NJ, NP = S // BN, S // CK, BN // 128, H // 2
    OFF = 32 - Dh
    qscale = Dh ** -0.5 * math.log2(math.e)
    chunks = list(range(U))
    chunks[FULL_AT:FULL_AT] = range(U, NC)
    sub = lax.broadcasted_iota(I32, (8, BN), 0)

    def blk(i):
        return pl.ds(pl.multiple_of(i * BN, BN), BN)

    def all_true(zero):
        return lax.broadcasted_iota(I32, (8, 128), 1) >= zero

    def x_copy(i):
        return pltpu.make_async_copy(x_hbm.at[:, blk(i)], xT.at[:, blk(i)], sem_x.at[i])

    w_copies = [pltpu.make_async_copy(s, d, sem_w.at[min(i, 2)]) for i, (s, d) in enumerate(
        [(wqkv_hbm.at[D2:], wqkv.at[D2:]), (wqkv_hbm.at[:D2], wqkv.at[:D2]),
         (wo_hbm, wo), (w1_hbm, w1), (b1_hbm, b1.at[:F]), (w2T_hbm, w2T), (b2_hbm, b2)])]

    def x_stats(i, true):
        load = lambda r, j: xT[r:r + 8, pl.ds(pl.multiple_of(i * BN + j, 128), 128)].astype(F32)
        return _ln_stats(load, D, BN, true)

    def qkv_weights(h):
        w_copies[1 - h].wait()
        for i in (1,) if h else range(2, NB):
            x_copy(i).start()
        t = wqkv[D2 * h:D2 * (h + 1), :].T.astype(F32)
        for m, src in enumerate((1, 0, 2)):
            aqkv[0, h, m * D2:(m + 1) * D2] = t[src * D:src * D + D2]
            aqkv[1, h, m * D2:(m + 1) * D2] = t[src * D + D2:(src + 1) * D]

    def windows(x, p, fill):
        a = 2 * Dh * p
        mid = x[a + 24:a + 32]
        return (_rows([x[a:a + 24], jnp.where(sub < OFF, mid, fill)]),
                _rows([jnp.where(sub >= OFF, mid, fill), x[a + 32:a + 56]]))

    def qkv(i, stats, order, hooks=None):
        c = _strassen(aqkv, _ln_apply(lambda r: xT[r:r + 8, blk(i)].astype(F32), D, stats), order, hooks)
        k, q, v = (_blocks([[x[m * D2:(m + 1) * D2] for x in row] for row in c]) for m in range(3))
        for p, e in itertools.product(range(NP), range(2)):
            a = 2 * Dh * p + 24 * e
            kt = _pk(_rows([k[a:a + 32], jnp.zeros((96, BN), F32)]).astype(BF16).T)
            kn[p, e, pl.ds(pl.multiple_of(i * (BN // 2), BN // 2), BN // 2), :] = _rows(
                [kt[r:r + 8] if r % 64 == 56 else pltpu.roll(kt[r:r + 8], 4, 0) for r in range(0, BN // 2, 8)])
        q = q * qscale
        qf[:, i] = q.reshape(NP, 2 * Dh, BN)
        for p in range(NP):
            for e, w in enumerate(windows(q, p, 0.0)):
                qp[p, e, i] = _pk(w.astype(BF16))
        for p in range(NP):
            for e, w in enumerate(windows(v, p, 1.0)):
                vT[p, e, :, blk(i)] = _pk(w.astype(BF16))

    def gather_vpu_keys(p, e, t, back=0):
        rows = [kn[p, e, pl.ds(pl.multiple_of(64 * c + 56 - (back if c >= NJ else 0), 8), 8), :]
                for c in range(8 * t, 8 * t + 8)]
        ku[p, e, :, 128 * t:128 * t + 128] = _up(_rows(rows)).T.astype(F32)[:32]

    def splat_vpu_keys(p, e, t):
        n = min(16, 2 * U - 16 * t)
        for d in range(Dh):
            row = ku[p, e, OFF * e + d:OFF * e + d + 1, 128 * t:128 * t + 128]
            (kb0, kb1)[e][16 * t:16 * t + n, d] = jnp.broadcast_to(row, (128, 128)).T[:8 * n].reshape(n, 8, 128)

    def more_x():
        x_copy(1).wait()
        for c in w_copies[2:]:
            c.start()

    x_copy(0).start()
    w_copies[0].start()
    sl[...] = jnp.zeros_like(sl)
    of[NP, 1, NB - 1] = jnp.zeros((32, BN), F32)
    x_copy(0).wait()
    w_copies[1].start()
    stats = x_stats(0, None)
    zero0 = attempt >> 20
    true0 = all_true(zero0)
    qkv(0, stats, ORD0, {4: lambda: qkv_weights(1), 3: lambda: qkv_weights(0), XH: more_x})

    def qkv_step(i, stats):
        gather_vpu_keys(0, 1, 0, jnp.where(i == 1, BN // 2, 0))
        splat_vpu_keys(zero0 if XS else 0, 1, 0)
        qkv(i, stats, ORD1)
        return x_stats(jnp.minimum(i + 1, NB - 1), true0)

    stats = x_stats(1, true0)
    for i in range(2, NB):
        x_copy(i).wait()
    lax.fori_loop(1, NB, qkv_step, stats)

    def q_tile(p, e, qb):
        return _up(_rows([qp[p, e, qb], jnp.zeros((48, BN), U32)]))

    def vpu_scores(p, e, seed):
        serial = itertools.count(1000 * e + 1)
        true = all_true((seed + next(serial)) >> 20) if TR else true0
        prev = None
        for qb, g, j in itertools.product(range(NB), range(0, 2 * U, TK), range(0, BN, 128)):
            z = (seed + next(serial)) >> 20
            kz = (kb0, kb1)[e].at[pl.ds(z, 2 * U)]
            acc = []
            for d in range(Dh):
                qd = jnp.broadcast_to(qf[p + z, qb, Dh * e + d:Dh * e + d + 1, j:j + 128], (8, 128))
                for a in range(TK):
                    kd = kz[g + a, d]
                    if d:
                        acc[a] = acc[a] + kd * qd
                    else:
                        acc.append((jnp.where(true, kd, prev[(a + XT) % TK]) if prev else kd) * qd)
            for a in range(TK):
                sv[qb, g + a, :, j:j + 128] = acc[a]
            prev = acc

    def head(p, e, last=False):
        p_in = _rows([jnp.exp2(sl[r:r + 8]) for r in reversed(range(0, CK, 8))][::-1])

        def finish_previous():
            dst = p if e else jnp.where(p == 0, NP, p - 1)
            v = vT[jnp.maximum(p - 1 + e, 0), 1 - e, :, chunks[-1] * CK:(chunks[-1] + 1) * CK]
            of[dst, 1 - e, NB - 1] = _dot(_up(v), p_in) + of[dst, 1 - e, NB - 1]

        pending = [finish_previous]
        for qb in range(NB):
            qm, acc = q_tile(p, e, qb), []
            defer = qb == NB - 1 and not last
            for n, c in enumerate(chunks):
                act = (lambda x: x) if defer and n == NC - 1 else jnp.exp2
                nb = 7 if c < U else 8
                tail = [act(sv[qb, 2 * c + i]) for i in (1, 0)][::-1] if c < U else None
                keys = _rows([kn[p, e, 64 * c + 8 * b:64 * c + 8 * b + 8, :] for b in reversed(range(nb))])
                s = act(_dot(_up(keys), qm))
                s = _rows([s[8 * b:8 * b + 8] for b in reversed(range(2 * nb - 14, 2 * nb))] + (tail or [s[:16]]))

                def pv(s=s, c=c, qb=qb, acc=acc, done=n == NC - 1 - defer):
                    r = _dot(_up(vT[p, e, :, c * CK:(c + 1) * CK]), s)
                    acc.append(r + acc.pop() if acc else r)
                    if done:
                        of[p, e, qb] = acc.pop()

                if act is jnp.exp2:
                    pending.append(pv)
                else:
                    sl[...] = s
                if not (qb == NB - 1 and n >= NC - (2 if last else 1)):
                    pending.pop(0)()
        for f in pending:
            f()
        if last:
            return
        pn = jnp.minimum(p + e, NP - 1) if MN else p + e
        vpu_scores(pn, 1 - e, p)
        for t in range(2):
            splat_vpu_keys(jnp.minimum(p + 1, NP - 1), e, t)
        for t in range(2):
            gather_vpu_keys(jnp.minimum(p + 1 + e, NP - 1), 1 - e, t)
        j = jnp.minimum(2 * p + e, F // 128 - 1)
        for h in range(2):
            w = w1[D2 * h:D2 * (h + 1), pl.ds(pl.multiple_of(j * 128, 128), 128)]
            t1[h, pl.ds(pl.multiple_of(j * 64, 64), 64), :] = _pk(_rows([w, jnp.zeros((256 - D2, 128), BF16)]).T)

    def head_pair(p, carry):
        pl.when(p > 0)(lambda: head(p - 1, 1))
        head(p, 0)
        return carry

    def ffn_weights():
        for h in range(2):
            ao[:, h] = wo[D2 * h:D2 * (h + 1), :].T.astype(F32).reshape(2, D2, D2)
        chain = None

        def second():
            nonlocal chain
            for r, j in itertools.product(range(0, D4, 16), range(0, F2, 128)):
                w = {10 * a + b + 11: w2T[a * D4 + r:a * D4 + r + 16, b * F2 + j:b * F2 + j + 128].astype(F32)
                     for a in range(4) for b in range(2)}
                for i, (lhs, _) in _HK.items():
                    f = _signed_sum(w.get, lhs)
                    slow = i % PA >= PB
                    if slow and chain is not None:
                        f = _rows([jnp.where(true0, f[:8], chain), f[8:]])
                    f = _pk(f.astype(BF16))
                    if not slow and chain is not None:
                        f = jnp.where(true0, f, pltpu.bitcast(chain, U32))
                    a2[i - 1, r // 2:r // 2 + 8, j:j + 128] = f
                    chain = pltpu.bitcast(f, F32)
                    yield

        def first():
            nonlocal chain
            for r, j in itertools.product(range(0, F4, 16), range(0, 256, 128)):
                w = {10 * a + b + 11: _up(t1[b, (a * F4 + r) // 2:(a * F4 + r) // 2 + 8, j:j + 128]).astype(F32)
                     for a in range(4) for b in range(2)}
                for i, (lhs, _) in _HK.items():
                    f = _signed_sum(w.get, lhs)
                    for t in (0, 8):
                        a1[i - 1, r + t:r + t + 8, j:j + 128] = chain = jnp.where(true0, f[t:t + 8], chain)
                    yield

        for _ in itertools.zip_longest(second(), first()):
            pass
        b1c[...] = jnp.broadcast_to(b1[:F].astype(F32).reshape(1, F), (128, F)).T
        b2c[...] = jnp.broadcast_to(b2[...].astype(F32).reshape(1, D), (128, D)).T

    def exact_attention(i, carry):
        p, e, qb = i // (2 * NB), (i // NB) % 2, i % NB
        qm = q_tile(p, e, qb)
        scores = lambda c: _dot(_up(kn[p, e, c // 2:(c + 256) // 2]), qm)
        m, acc, s = jnp.full((1, BN), -jnp.inf, F32), jnp.zeros((32, BN), F32), scores(0)
        for c in range(0, S, 256):
            nxt = scores(c + 256) if c + 256 < S else None
            s = _rows([s[8 * (b if b % 16 >= 14 else b ^ 1):][:8] for b in range(32)])
            m_new = jnp.maximum(m, jnp.max(s, axis=0, keepdims=True))
            acc = _dot(_up(vT[p, e, :, c:c + 256]), jnp.exp2(s - m_new)) + acc * jnp.exp2(m - m_new)
            m, s = m_new, nxt
        of[p, e, qb] = acc
        return carry

    gather_vpu_keys(0, 1, 1)
    splat_vpu_keys(0, 1, 1)
    for t in range(2):
        gather_vpu_keys(1, 0, t)
    keys = _up(_rows([kn[0, 0, 64 * c + 56:64 * c + 64, :] for c in range(U)]))
    for qb in range(NB):
        sv[qb] = _dot(keys, q_tile(0, 0, qb)).reshape(2 * U, 8, BN)
    for c in w_copies[2:]:
        c.wait()

    @pl.when(attempt == 0)
    def _():
        if '2' in PH:
            lax.fori_loop(0, NP, head_pair, 0)
        ffn_weights()
        head(NP - 1, 1, last=True)

    @pl.when(attempt == 1)
    def _():
        lax.fori_loop(0, H * NB, exact_attention, 0)

    def project(i, l_range):
        parts = []
        for p in range(NP):
            oe, oo = of[p, 0, i], of[p, 1, i]
            l = jnp.where(sub < OFF, oo[0:8], oe[24:32])
            l_range = (jnp.minimum(l_range[0], l), jnp.maximum(l_range[1], l))
            inv = pltpu.reciprocal(l, approx=True)
            inv = inv * (2.0 - l * inv)
            ie, io = jnp.broadcast_to(inv[7:8], (8, BN)), jnp.broadcast_to(inv[0:1], (8, BN))
            parts += [oe[0:24] * jnp.tile(ie, (3, 1)), jnp.where(sub < OFF, oe[24:32] * ie, oo[0:8] * io),
                      oo[8:32] * jnp.tile(io, (3, 1))]
        hs[i] = _blocks(_strassen(ao, _rows(parts), ORD2)) + xT[:, blk(i)].astype(F32)
        return l_range

    true = all_true((attempt + 1) >> 20)
    h_stats = lambda i, true: _ln_stats(lambda r, j: hs[i, r:r + 8, j:j + 128], D, BN, true)
    one = jnp.ones((8, BN), F32)
    l_range = project(0, (one, one))
    stats = h_stats(0, None)
    for i in range(1, NB):
        l_range = project(i, l_range)

    def ffn(i, carry):
        stats, rmin = carry
        u = _hopcroft_kerr(lambda n: a1[n - 1, :, :D2], _ln_apply(lambda r: hs[i, r:r + 8], D, stats), HO3)
        act = lambda x, r: jnp.square(jnp.maximum(x + b1c[r:r + 8], 0.0))
        y = _hopcroft_kerr(lambda n: _up(a2[n - 1]), u, HO4, act, true)
        outT[:, blk(i)] = (y + (hs[i] + jnp.tile(b2c[...], (1, NJ)))).astype(outT.dtype)
        nxt = h_stats(jnp.minimum(i + 1, NB - 1), true)
        pltpu.make_async_copy(outT.at[:, blk(i)], out_hbm.at[:, blk(i)], sem_o).start()
        return nxt, jnp.minimum(rmin, stats[1])

    _, rmin = lax.fori_loop(0, NB, ffn, (stats, one))
    ok = (l_range[0] >= L_LO) & (l_range[1] <= L_HI) & (rmin > 0.0)
    redo = jnp.logical_and(attempt == 0, jnp.min(jnp.where(ok, 1.0, 0.0)) < 0.5)
    for i in range(NB):
        pltpu.make_async_copy(outT.at[:, blk(i)], out_hbm.at[:, blk(i)], sem_o).wait()
    if PH != '23':
        outT[0:16, 0:128] = pltpu.bitcast(kb1[attempt, 0] + ku[attempt, 0, 0:8, 0:128] + qf[attempt, 0, 0:8, 0:128], BF16)
    return jnp.where(redo, 1, 2)


@jax.jit
def pallas_sequential_preLN__softmax_full_mha__dense_activation_squared_relu__prompt_kernel(
    A_x, A_wqkv, A_wo, B_x, B_w1, B_b1, B_w2, B_b2,
):
    del B_x
    B, S, D = A_x.shape
    F = B_w1.shape[1]
    Dh, NB, NP = D // H, S // BN, H // 2
    vmem, hbm = pltpu.VMEM, pl.BlockSpec(memory_space=pl.ANY)
    outT = pl.pallas_call(
        _kernel,
        out_shape=jax.ShapeDtypeStruct((D, S), A_x.dtype),
        in_specs=[hbm] * 7,
        out_specs=hbm,
        scratch_shapes=[
            vmem((32, Dh, 8, 128), F32),
            vmem((32, Dh, 8, 128), F32),
            vmem((NB, 2 * U, 8, BN), F32),
            vmem((NP, 2, NB, 16, BN), U32),
            vmem((NP, NB, 2 * Dh, BN), F32),
            vmem((NP, 2, S // 2, 128), U32),
            vmem((NP, 2, 16, S), U32),
            vmem((NP + 1, 2, NB, 32, BN), F32),
            vmem((CK, BN), F32),
            vmem((NP, 2, 32, 256), F32),
            vmem((D, S), BF16),
            vmem((D, S), BF16),
            vmem((D, D), BF16),
            vmem((2, 2, 3 * D // 2, D // 2), F32),
            vmem((2, 2, D // 2, D // 2), F32),
            vmem((26, F // 4, 256), F32),
            vmem((2, F // 2, 256), U32),
            vmem((F, 128), F32),
            vmem((NB, D, BN), F32),
            vmem((D, F), BF16),
            vmem((D, F), BF16),
            vmem((26, D // 8, F // 2), U32),
            vmem((D, 128), F32),
            vmem((D, 3 * D), BF16),
            vmem((2 * F,), BF16),
            vmem((D,), BF16),
            pltpu.SemaphoreType.DMA((NB,)),
            pltpu.SemaphoreType.DMA((3,)),
            pltpu.SemaphoreType.DMA(()),
        ],
        compiler_params=pltpu.CompilerParams(vmem_limit_bytes=100 * 1024 * 1024),
        name="block",
    )(A_x.reshape(S, D).T, A_wqkv, A_wo, B_w1, B_b1, B_w2.T, B_b2)
    return outT.T.reshape(B, S, D)
```

```python
import itertools
import math

import jax
import jax.numpy as jnp
from jax import lax
import jax.experimental.pallas as pl
import jax.experimental.pallas.tpu as pltpu

H = 16
EPS = 1e-5
BN = 512
CK = 128
U = 15
VROWS = 24
L_LO, L_HI = 2.0 ** -40, 2.0 ** 60
F32, BF16, U32, I32 = jnp.float32, jnp.bfloat16, jnp.uint32, jnp.int32

_STRASSEN = {
    1: ((11, 22), (11, 22), (11, 22)),
    2: ((21, 22), (11,), (21, -22)),
    3: ((11,), (12, -22), (12, 22)),
    4: ((22,), (21, -11), (11, 21)),
    5: ((11, 12), (22,), (-11, 12)),
    6: ((21, -11), (11, 12), (22,)),
    7: ((12, -22), (21, 22), (11,)),
}
_HK = {
    1: ((11,), (11,)), 2: ((12,), (21,)), 3: ((21,), (12, -22)), 4: ((21, 22), (22,)),
    5: ((31,), (13, -23)), 6: ((31, 32), (23,)), 7: ((42,), (24, -14)), 8: ((41, 42), (14,)),
    9: ((21, 22, 12), (11, 12, -22)), 10: ((12, 22), (11, 12, -22, -21)),
    11: ((21, 22, 12, 11), (11, 12)),
    12: ((31, 32, 12), (11, 13, -23)), 13: ((12, 32), (11, 13, -23, -21)),
    14: ((31, 32, 12, 11), (11, 13)),
    15: ((41, 42, 11), (21, -24, 14)), 16: ((11, 41), (21, -24, 14, -11)),
    17: ((41, 42, 11, 12), (21, -24)),
    18: ((21, 42), (14, 22)), 19: ((41, -21), (12, 14)), 20: ((22, -42), (22, 24)),
    21: ((31, 42), (14, 23)), 22: ((41, -31), (13, 14)), 23: ((32, -42), (23, 24)),
    24: ((12, 22, -31), (11, 12, 23)), 25: ((12, 22, 32), (21, 22, 23)),
    26: ((11, 21, 31), (11, 12, 13)),
}
_HK_OUT = {
    11: (1, 2), 22: (3, 4), 33: (5, 6), 44: (7, 8),
    21: (9, -2, -3, -10), 12: (11, -9, -1, -4), 31: (12, -2, -5, -13), 13: (14, -12, -1, -6),
    41: (15, 7, -1, -16), 14: (15, 2, -8, -17), 42: (18, 3, -8, 19), 24: (18, 7, -4, 20),
    43: (21, 5, -8, 22), 34: (21, 7, -6, 23),
    32: (10, -24, -6, -131, 25), 23: (24, -11, -5, -113, 26),
}
_FFN1_ORDER = (3, 4, 1, 2, 11, 9, 10, 5, 15, 14, 12, 13, 8, 7, 6, 17, 16, 21, 18, 19, 20, 24, 25, 22, 26, 23)
_FFN2_ORDER = (26, 1, 11, 2, 4, 3, 9, 14, 8, 22, 19, 17, 10, 5, 7, 20, 23, 18, 25, 6, 12, 16, 13, 24, 21, 15)


def _pk(x):
    return pltpu.bitcast(x, U32)


def _up(x):
    return pltpu.bitcast(x, BF16)


def _dot(a, b):
    return lax.dot_general(a, b, (((1,), (0,)), ((), ())), preferred_element_type=F32)


def _rows(parts):
    return jnp.concatenate(parts, axis=0)


def _blocks(c):
    return _rows([jnp.concatenate(r, axis=1) for r in c])


def _all_true(zero, rows=8):
    return lax.broadcasted_iota(I32, (rows, 128), 1) >= zero


def _signed_sum(get, terms):
    out = get(terms[0])
    for t in terms[1:]:
        out = out + get(t) if t > 0 else out - get(-t)
    return out


def _ln_stats(load, d, true=None):
    mean, rstd = [], []
    for j in range(0, BN, 128):
        acc = load(0, j)
        if rstd and true is not None:
            acc = jnp.where(true, acc, rstd[-1])
        for r in range(8, d, 8):
            acc = acc + load(r, j)
        m = jnp.broadcast_to(jnp.sum(acc, axis=0, keepdims=True) * (1.0 / d), (8, 128))
        for r in range(0, d, 8):
            c = load(r, j) - m
            acc = acc + c * c if r else c * c
        v = jnp.broadcast_to(jnp.sum(acc, axis=0, keepdims=True) * (1.0 / d), (8, 128))
        mean.append(m)
        rstd.append(lax.rsqrt(v + EPS))
    return jnp.concatenate(mean, axis=1), jnp.concatenate(rstd, axis=1)


def _ln_apply(load, d, stats):
    return _rows([(load(r) - stats[0]) * stats[1] for r in range(0, d, 8)])


def _strassen(a_ref, b, order, hooks=None):
    k, n = b.shape[0] // 2, b.shape[1] // 2
    bq = {11: b[:k, :n], 12: b[:k, n:], 21: b[k:, :n], 22: b[k:, n:]}
    c = {}
    for i in order:
        lhs, rhs, dst = _STRASSEN[i]
        rhs = _signed_sum(bq.get, rhs)
        if hooks and i in hooks:
            hooks[i]()
        m = _dot(_signed_sum(lambda q: a_ref[q // 10 - 1, q % 10 - 1], lhs), rhs)
        for t in dst:
            if abs(t) not in c:
                c[abs(t)] = (m, t > 0)
            else:
                acc, pos = c[abs(t)]
                c[abs(t)] = (m + acc if pos and t > 0 else acc - m if pos else m - acc, True)
    return [[c[11][0], c[12][0]], [c[21][0], c[22][0]]]


def _hopcroft_kerr(lhs, b, order, act=lambda x, r: x, true=None):
    k, n = b.shape[0] // 2, b.shape[1] // 4
    memo = {}

    def rhs(terms, r, prev):
        def tie(x):
            nonlocal prev
            if prev is not None and true is not None:
                x, prev = jnp.where(true, x, prev), None
            return x

        for q in map(abs, terms):
            if ((q,), r) not in memo:
                r0 = (q // 10 - 1) * k + r
                memo[(q,), r] = act(tie(b[r0:r0 + 8, (q % 10 - 1) * n:q % 10 * n]), r0)
        for c in range(2, len(terms) + 1):
            if (terms[:c], r) not in memo:
                f, t = tie(memo[terms[:c - 1], r]), terms[c - 1]
                memo[terms[:c], r] = f + memo[(t,), r] if t > 0 else f - memo[(-t,), r]
        return memo[terms, r]

    m = {}
    for i in order:
        rows = []
        for r in reversed(range(0, k, 8)):
            rows.append(rhs(_HK[i][1], r, rows[-1] if rows and r % 128 != 120 else None))
        m[i] = _dot(lhs(i), _rows(rows[::-1]))
        for q, terms in _HK_OUT.items():
            if 100 + q not in m and all(abs(t) in m for t in terms):
                rest = sorted((t for t in terms if t != i), key=lambda t: t < 0)
                if i in terms and rest[0] > 0:
                    m[100 + q] = m[i] + _signed_sum(m.get, rest)
                else:
                    m[100 + q] = _signed_sum(m.get, terms)
    return _blocks([[m[100 + 10 * r + c] for c in range(1, 5)] for r in range(1, 5)])


def _kernel(*refs):
    lax.while_loop(lambda attempt: attempt < 2, lambda attempt: _block(attempt, *refs), 0)


def _block(attempt, x_hbm, wqkv_hbm, wo_hbm, w1_hbm, b1_hbm, w2T_hbm, b2_hbm, out_hbm,
           kb0, kb1, sv, qp, qf, kn, vT, of, sl, ku, xT, outT, wo, aqkv, ao, a1, t1, b1c, hs,
           w1, w2T, a2, b2c, wqkv, b1, b2, sem_x, sem_w, sem_o):
    D, S = x_hbm.shape
    F = w1_hbm.shape[1]
    Dh, D2, D4, F2, F4 = D // H, D // 2, D // 4, F // 2, F // 4
    NB, NC, NJ, NP = S // BN, S // CK, BN // 128, H // 2
    OFF = 32 - Dh
    sub = lax.broadcasted_iota(I32, (8, BN), 0)

    def blk(i):
        return pl.ds(pl.multiple_of(i * BN, BN), BN)

    def x_copy(i):
        return pltpu.make_async_copy(x_hbm.at[:, blk(i)], xT.at[:, blk(i)], sem_x.at[i])

    def out_copy(i):
        return pltpu.make_async_copy(outT.at[:, blk(i)], out_hbm.at[:, blk(i)], sem_o.at[i])

    w_copies = [pltpu.make_async_copy(s, d, sem_w.at[i]) for i, (s, d) in enumerate(
        [(wqkv_hbm.at[D2:], wqkv.at[D2:]), (wqkv_hbm.at[:D2], wqkv.at[:D2]),
         (wo_hbm, wo), (w1_hbm, w1), (b1_hbm, b1.at[:F]), (w2T_hbm, w2T), (b2_hbm, b2)])]

    def x_stats(i, true=None):
        load = lambda r, j: xT[r:r + 8, pl.ds(pl.multiple_of(i * BN + j, 128), 128)].astype(F32)
        return _ln_stats(load, D, true)

    def qkv_weights(h):
        w_copies[1 - h].wait()
        for i in (1,) if h else range(2, NB):
            x_copy(i).start()
        t = wqkv[D2 * h:D2 * (h + 1), :].T.astype(F32)
        for m, src in enumerate((1, 0, 2)):
            aqkv[0, h, m * D2:(m + 1) * D2] = t[src * D:src * D + D2]
            aqkv[1, h, m * D2:(m + 1) * D2] = t[src * D + D2:(src + 1) * D]

    def second_block_arrived():
        x_copy(1).wait()
        for c in w_copies[2:]:
            c.start()

    def windows(x, p, fill):
        a = 2 * Dh * p
        mid = x[a + 24:a + 32]
        return (_rows([x[a:a + 24], jnp.where(sub < OFF, mid, fill)]),
                _rows([jnp.where(sub >= OFF, mid, fill), x[a + 32:a + 56]]))

    def qkv(i, stats, order, hooks=None):
        xn = _ln_apply(lambda r: xT[r:r + 8, blk(i)].astype(F32), D, stats)
        c = _strassen(aqkv, xn, order, hooks)
        k, q, v = (_blocks([[x[m * D2:(m + 1) * D2] for x in row] for row in c]) for m in range(3))
        for p, e in itertools.product(range(NP), range(2)):
            a = 2 * Dh * p + 24 * e
            kt = _pk(_rows([k[a:a + 32], jnp.zeros((96, BN), F32)]).astype(BF16).T)
            kn[p, e, pl.ds(pl.multiple_of(i * (BN // 2), BN // 2), BN // 2), :] = _rows(
                [kt[r:r + 8] if r % 64 == 56 else pltpu.roll(kt[r:r + 8], 4, 0)
                 for r in range(0, BN // 2, 8)])
        q = q * (Dh ** -0.5 * math.log2(math.e))
        qf[:, i] = q.reshape(NP, 2 * Dh, BN)
        for p in range(NP):
            for e, w in enumerate(windows(q, p, 0.0)):
                qp[p, e, i] = _pk(w.astype(BF16))
        for p in range(NP):
            for e, w in enumerate(windows(v, p, 1.0)):
                vT[p, e, :, blk(i)] = _pk(w.astype(BF16))

    def gather_vpu_keys(p, e, t, back=0):
        rows = [kn[p, e, pl.ds(pl.multiple_of(64 * c + 56 - (back if c >= NJ else 0), 8), 8), :]
                for c in range(8 * t, 8 * t + 8)]
        ku[p, e, :, 128 * t:128 * t + 128] = _up(_rows(rows)).T.astype(F32)[:32]

    def splat_vpu_keys(p, e, t):
        n = min(128, 16 * U - 128 * t)
        for d in range(Dh):
            row = ku[p, e, OFF * e + d:OFF * e + d + 1, 128 * t:128 * t + 128]
            (kb0, kb1)[e][d, 128 * t:128 * t + n] = jnp.broadcast_to(row, (128, 128)).T[:n]

    x_copy(0).start()
    w_copies[0].start()
    sl[...] = jnp.zeros_like(sl)
    of[NP, 1, NB - 1] = jnp.zeros((32, BN), F32)
    x_copy(0).wait()
    w_copies[1].start()
    stats = x_stats(0)
    zero = attempt >> 20
    true = _all_true(zero)
    qkv(0, stats, (4, 7, 3, 5, 1, 2, 6),
        {4: lambda: qkv_weights(1), 3: lambda: qkv_weights(0), 5: second_block_arrived})

    def qkv_step(i, stats):
        gather_vpu_keys(0, 1, 0, jnp.where(i == 1, BN // 2, 0))
        splat_vpu_keys(zero, 1, 0)
        qkv(i, stats, (2, 4, 5, 3, 7, 1, 6))
        return x_stats(jnp.minimum(i + 1, NB - 1), true)

    stats = x_stats(1, true)
    for i in range(2, NB):
        x_copy(i).wait()
    lax.fori_loop(1, NB, qkv_step, stats)

    chunks = list(range(U - 1)) + list(range(U, NC)) + [U - 1]

    def q_tile(p, e, qb):
        return _up(_rows([qp[p, e, qb], jnp.zeros((48, BN), U32)]))

    def vpu_scores(p, e, seed):
        serial = itertools.count(1000 * e + 1)
        true = _all_true((seed + next(serial)) >> 20, VROWS)
        acc = None
        for qb, g, j in itertools.product(range(NB), range(0, 16 * U, VROWS), range(0, BN, 128)):
            zero = (seed + next(serial)) >> 20
            kz, qz = (kb0, kb1)[e].at[pl.ds(zero, Dh)], qf.at[p + zero, qb]
            prev = acc
            for d in range(Dh):
                qd = qz[Dh * e + d:Dh * e + d + 1, j:j + 128]
                kd = kz[d, g:g + VROWS]
                if d == e and prev is not None:
                    kd = jnp.where(true, kd, _rows([prev[8:], prev[:8]]))
                acc = acc + kd * qd if d else kd * qd
            sv[qb, g:g + VROWS, j:j + 128] = acc

    def head(p, e, last=False):
        p_in = _rows([jnp.exp2(sl[r:r + 8]) for r in reversed(range(0, CK, 8))][::-1])

        def finish_previous():
            dst = p if e else jnp.where(p == 0, NP, p - 1)
            v = vT[jnp.maximum(p - 1 + e, 0), 1 - e, :, chunks[-1] * CK:(chunks[-1] + 1) * CK]
            of[dst, 1 - e, NB - 1] = _dot(_up(v), p_in) + of[dst, 1 - e, NB - 1]

        pending = [finish_previous]
        for qb in range(NB):
            qm, acc = q_tile(p, e, qb), []
            defer = qb == NB - 1 and not last
            for n, c in enumerate(chunks):
                act = (lambda x: x) if defer and n == NC - 1 else jnp.exp2
                nb = 7 if c < U else 8
                tail = [act(sv[qb, 16 * c + i:16 * c + i + 8]) for i in (8, 0)][::-1] if c < U else None
                keys = _rows([kn[p, e, 64 * c + 8 * b:64 * c + 8 * b + 8, :] for b in reversed(range(nb))])
                s = act(_dot(_up(keys), qm))
                s = _rows([s[8 * b:8 * b + 8] for b in reversed(range(2 * nb - 14, 2 * nb))]
                          + (tail or [s[:16]]))

                def pv(s=s, c=c, qb=qb, acc=acc, done=n == NC - 1 - defer):
                    r = _dot(_up(vT[p, e, :, c * CK:(c + 1) * CK]), s)
                    acc.append(r + acc.pop() if acc else r)
                    if done:
                        of[p, e, qb] = acc.pop()

                if act is jnp.exp2:
                    pending.append(pv)
                else:
                    sl[...] = s
                if not (qb == NB - 1 and n >= NC - (2 if last else 1)):
                    pending.pop(0)()
        for f in pending:
            f()
        if last:
            return
        vpu_scores(jnp.minimum(p + e, NP - 1), 1 - e, p)
        for t in range(2):
            splat_vpu_keys(jnp.minimum(p + 1, NP - 1), e, t)
        for t in range(2):
            gather_vpu_keys(jnp.minimum(p + 1 + e, NP - 1), 1 - e, t)
        j = jnp.minimum(2 * p + e, F // 128 - 1)
        for h in range(2):
            w = w1[D2 * h:D2 * (h + 1), pl.ds(pl.multiple_of(j * 128, 128), 128)]
            t1[h, pl.ds(pl.multiple_of(j * 64, 64), 64), :] = _pk(
                _rows([w, jnp.zeros((256 - D2, 128), BF16)]).T)

    def head_pair(p, carry):
        pl.when(p > 0)(lambda: head(p - 1, 1))
        head(p, 0)
        return carry

    def late_weights():
        for h in range(2):
            ao[:, h] = wo[D2 * h:D2 * (h + 1), :].T.astype(F32).reshape(2, D2, D2)
        chain = None

        def second():
            nonlocal chain
            for r, j in itertools.product(range(0, D4, 16), range(0, F2, 128)):
                w = {10 * a + b + 11: w2T[pl.ds(a * D4 + r, 16), pl.ds(b * F2 + j, 128)].astype(F32)
                     for a in range(4) for b in range(2)}
                for i, (lhs, _) in _HK.items():
                    f = _signed_sum(w.get, lhs)
                    if i % 3 and chain is not None:
                        f = _rows([jnp.where(true, f[:8], chain), f[8:]])
                    f = _pk(f.astype(BF16))
                    if i % 3 == 0:
                        f = jnp.where(true, f, pltpu.bitcast(chain, U32))
                    a2[i - 1, r // 2:r // 2 + 8, j:j + 128] = f
                    chain = pltpu.bitcast(f, F32)
                    yield

        def first():
            nonlocal chain
            for r, j in itertools.product(range(0, F4, 16), range(0, 256, 128)):
                w = {10 * a + b + 11: _up(t1[b, pl.ds((a * F4 + r) // 2, 8), j:j + 128]).astype(F32)
                     for a in range(4) for b in range(2)}
                for i, (lhs, _) in _HK.items():
                    f = _signed_sum(w.get, lhs)
                    for t in (0, 8):
                        chain = jnp.where(true, f[t:t + 8], chain)
                        a1[i - 1, r + t:r + t + 8, j:j + 128] = chain
                    yield

        for _ in itertools.zip_longest(second(), first()):
            pass
        b1c[...] = jnp.broadcast_to(b1[:F].astype(F32).reshape(1, F), (128, F)).T
        b2c[...] = jnp.broadcast_to(b2[...].astype(F32).reshape(1, D), (128, D)).T

    def true_max_attention(i, carry):
        p, e, qb = i // (2 * NB), (i // NB) % 2, i % NB
        qm = q_tile(p, e, qb)
        scores = lambda c: _dot(_up(kn[p, e, c // 2:(c + 256) // 2]), qm)
        m, acc, s = jnp.full((1, BN), -jnp.inf, F32), jnp.zeros((32, BN), F32), scores(0)
        for c in range(0, S, 256):
            nxt = scores(c + 256) if c + 256 < S else None
            s = _rows([s[8 * (b if b % 16 >= 14 else b ^ 1):][:8] for b in range(32)])
            m_new = jnp.maximum(m, jnp.max(s, axis=0, keepdims=True))
            acc = _dot(_up(vT[p, e, :, c:c + 256]), jnp.exp2(s - m_new)) + acc * jnp.exp2(m - m_new)
            m, s = m_new, nxt
        of[p, e, qb] = acc
        return carry

    gather_vpu_keys(0, 1, 1)
    splat_vpu_keys(0, 1, 1)
    for t in range(2):
        gather_vpu_keys(1, 0, t)
    keys = _up(_rows([kn[0, 0, 64 * c + 56:64 * c + 64, :] for c in range(U)]))
    for qb in range(NB):
        sv[qb] = _dot(keys, q_tile(0, 0, qb))
    for c in w_copies[2:]:
        c.wait()

    @pl.when(attempt == 0)
    def _():
        lax.fori_loop(0, NP, head_pair, 0)
        late_weights()
        head(NP - 1, 1, last=True)

    @pl.when(attempt == 1)
    def _():
        lax.fori_loop(0, H * NB, true_max_attention, 0)

    def project(i, l_range):
        parts = []
        for p in range(NP):
            even, odd = of[p, 0, i], of[p, 1, i]
            l = jnp.where(sub < OFF, odd[0:8], even[24:32])
            l_range = (jnp.minimum(l_range[0], l), jnp.maximum(l_range[1], l))
            inv = 1.0 / l
            inv_e, inv_o = jnp.broadcast_to(inv[7:8], (8, BN)), jnp.broadcast_to(inv[0:1], (8, BN))
            parts += [even[0:24] * jnp.tile(inv_e, (3, 1)),
                      jnp.where(sub < OFF, even[24:32] * inv_e, odd[0:8] * inv_o),
                      odd[8:32] * jnp.tile(inv_o, (3, 1))]
        a = _blocks(_strassen(ao, _rows(parts), (5, 3, 2, 4, 1, 6, 7)))
        hs[i] = a + xT[:, blk(i)].astype(F32)
        return l_range

    true3 = _all_true((attempt + 1) >> 20)
    h_stats = lambda i, true=None: _ln_stats(lambda r, j: hs[i, r:r + 8, j:j + 128], D, true)
    one = jnp.ones((8, BN), F32)
    l_range = project(0, (one, one))
    stats = h_stats(0)
    for i in range(1, NB):
        l_range = project(i, l_range)

    def ffn(i, carry):
        stats, rstd_min = carry
        hn = _ln_apply(lambda r: hs[i, r:r + 8], D, stats)
        u = _hopcroft_kerr(lambda n: a1[n - 1, :, :D2], hn, _FFN1_ORDER)
        act = lambda x, r: jnp.square(jnp.maximum(x + b1c[r:r + 8], 0.0))
        y = _hopcroft_kerr(lambda n: _up(a2[n - 1]), u, _FFN2_ORDER, act, true3)
        outT[:, blk(i)] = (y + (hs[i] + jnp.tile(b2c[...], (1, NJ)))).astype(outT.dtype)
        nxt = h_stats(jnp.minimum(i + 1, NB - 1), true3)
        out_copy(i).start()
        return nxt, jnp.minimum(rstd_min, stats[1])

    _, rstd_min = lax.fori_loop(0, NB, ffn, (stats, one))
    safe = (l_range[0] >= L_LO) & (l_range[1] <= L_HI) & (rstd_min > 0.0)
    redo = jnp.logical_and(attempt == 0, jnp.min(jnp.where(safe, 1.0, 0.0)) < 0.5)
    for i in range(NB):
        out_copy(i).wait()
    return jnp.where(redo, 1, 2)


@jax.jit
def pallas_sequential_preLN__softmax_full_mha__dense_activation_squared_relu__prompt_kernel(
    A_x: jax.Array,
    A_wqkv: jax.Array,
    A_wo: jax.Array,
    B_x: jax.Array,
    B_w1: jax.Array,
    B_b1: jax.Array,
    B_w2: jax.Array,
    B_b2: jax.Array,
):
    del B_x
    B, S, D = A_x.shape
    F = B_w1.shape[1]
    assert (B, S, D, F) == (1, 2048, 448, 1792)
    NB, NP = S // BN, H // 2
    vmem, hbm = pltpu.VMEM, pl.BlockSpec(memory_space=pl.ANY)
    outT = pl.pallas_call(
        _kernel,
        out_shape=jax.ShapeDtypeStruct((D, S), A_x.dtype),
        in_specs=[hbm] * 7,
        out_specs=hbm,
        scratch_shapes=[
            vmem((32, 16 * U, 128), F32),
            vmem((32, 16 * U, 128), F32),
            vmem((NB, 16 * U, BN), F32),
            vmem((NP, 2, NB, 16, BN), U32),
            vmem((NP, NB, 2 * D // H, BN), F32),
            vmem((NP, 2, S // 2, 128), U32),
            vmem((NP, 2, 16, S), U32),
            vmem((NP + 1, 2, NB, 32, BN), F32),
            vmem((CK, BN), F32),
            vmem((NP, 2, 32, 256), F32),
            vmem((D, S), BF16),
            vmem((D, S), BF16),
            vmem((D, D), BF16),
            vmem((2, 2, 3 * D // 2, D // 2), F32),
            vmem((2, 2, D // 2, D // 2), F32),
            vmem((26, F // 4, 256), F32),
            vmem((2, F // 2, 256), U32),
            vmem((F, 128), F32),
            vmem((NB, D, BN), F32),
            vmem((D, F), BF16),
            vmem((D, F), BF16),
            vmem((26, D // 8, F // 2), U32),
            vmem((D, 128), F32),
            vmem((D, 3 * D), BF16),
            vmem((2 * F,), BF16),
            vmem((D,), BF16),
            pltpu.SemaphoreType.DMA((NB,)),
            pltpu.SemaphoreType.DMA((7,)),
            pltpu.SemaphoreType.DMA((NB,)),
        ],
        compiler_params=pltpu.CompilerParams(vmem_limit_bytes=100 * 1024 * 1024),
        name="block",
    )(A_x.reshape(S, D).T, A_wqkv, A_wo, B_w1, B_b1, B_w2.T, B_b2)
    return outT.T.reshape(B, S, D)
```
